```python
import os as _os
_os.environ.setdefault("JAX_PLATFORMS", "cpu")
import jax
import jax.numpy as jnp

def _softmax(x, axis=-1):
    return jax.nn.softmax(x, axis=axis)
def _gelu(x):
    return jax.nn.gelu(x, approximate=True)
def _silu(x):
    return jax.nn.silu(x)
def _sigmoid(x):
    return jax.nn.sigmoid(x)
def _layernorm(x, axis=-1, eps=1e-5):
    m = jnp.mean(x, axis=axis, keepdims=True)
    v = jnp.var(x, axis=axis, keepdims=True)
    return (x - m) / jnp.sqrt(v + eps)
def _scatter_add(tgt, idx, src, axis=0):
    return tgt.at[idx].add(src)
def _segment_sum(src, seg, n):
    return jax.ops.segment_sum(src, seg, n)
class _Rng:
    def __init__(self, key):
        self._k = key
    def _next(self):
        self._k, sub = jax.random.split(self._k)
        return sub
    def normal(self, shape):
        return jax.random.normal(self._next(), shape, dtype=jnp.bfloat16)
    def randint(self, lo, hi, shape):
        return jax.random.randint(self._next(), shape, lo, hi, dtype=jnp.int32)
    def uniform(self, shape, lo=0.0, hi=1.0):
        return jax.random.uniform(self._next(), shape, jnp.bfloat16, lo, hi)
    def permutation(self, n):
        return jax.random.permutation(self._next(), n)


kernel_name = 'sequential_preLN__softmax_full_mha__swiglu_ffn__prompt'

def setup_inputs():
    _rng = _Rng(jax.random.key(int.from_bytes(__import__("os").urandom(4), "little")))
    _w = (lambda a: (lambda t: t.astype(jnp.bfloat16) if jnp.issubdtype(t.dtype, jnp.floating) else t)(jnp.asarray(a)))
    def _A_setup():
        B, S, D = 1, 2048, 512
        return {
            "x": _w((lambda *s: _rng.normal(s) * 0.05)(B, S, D)),
            "wqkv": _w((lambda *s: _rng.normal(s) * 0.05)(D, 3 * D)),
            "wo": _w((lambda *s: _rng.normal(s) * 0.05)(D, D)),
        }
    _A_in = _A_setup()

    def _B_setup():
        B, S, D, F = 1, 2048, 512, 1792
        return {
            "x": _w((lambda *s: _rng.normal(s) * 0.05)(B, S, D)),
            "w_gate": _w((lambda *s: _rng.normal(s) * 0.05)(D, F)),
            "w_up": _w((lambda *s: _rng.normal(s) * 0.05)(D, F)),
            "w_down": _w((lambda *s: _rng.normal(s) * 0.05)(F, D)),
        }
    _B_in = _B_setup()

    return {
        "A_x": _A_in["x"],
        "A_wqkv": _A_in["wqkv"],
        "A_wo": _A_in["wo"],
        "B_x": _B_in["x"],
        "B_w_gate": _B_in["w_gate"],
        "B_w_up": _B_in["w_up"],
        "B_w_down": _B_in["w_down"],
    }

def reference(A_x, A_wqkv, A_wo, B_x, B_w_gate, B_w_up, B_w_down):
    def _A_ref(x, wqkv, wo):
        B, S, D = x.shape
        H = 32; Dh = D // H
        qkv = (lambda x, *d: x.transpose(*d))((x @ wqkv).reshape(B, S, 3, H, Dh), 2, 0, 3, 1, 4)
        q, k, v = qkv[0], qkv[1], qkv[2]
        scale = Dh ** -0.5
        scores = jnp.einsum("bhqd,bhkd->bhqk", q, k) * scale
        p = _softmax(scores, axis=-1)
        o = jnp.einsum("bhqk,bhkd->bhqd", p, v)
        return (lambda x, *d: x.transpose(*d))(o, 0, 2, 1, 3).reshape(B, S, D) @ wo

    def _B_ref(x, w_gate, w_up, w_down):
        g = _silu(x @ w_gate)
        u = x @ w_up
        return (g * u) @ w_down

    x = A_x
    h = x + _A_ref(_layernorm(x, axis=-1), A_wqkv, A_wo)
    h2 = h + _B_ref(_layernorm(h, axis=-1), B_w_gate, B_w_up, B_w_down)
    return h2
```

```python
import functools
import math

import jax
import jax.numpy as jnp
from jax import lax
import jax.experimental.pallas as pl
import jax.experimental.pallas.tpu as pltpu

S, D, H, DH, F = 2048, 512, 32, 16, 1792
EPS = 1e-5

TQ = 512
NQ = S // TQ
CK = 128
NC = S // CK
NS = 2
LAG = 3
TM = 512
NT = S // TM
FC = 256
NF = F // FC
HPG = 128 // DH
QSCALE = (DH ** -0.5) * math.log2(math.e)

_f32 = jnp.float32
_bf16 = jnp.bfloat16


def _layernorm(x):
    m = jnp.mean(x, axis=-1, keepdims=True)
    xc = x - m
    v = jnp.mean(xc * xc, axis=-1, keepdims=True)
    return xc * lax.rsqrt(v + EPS)


def _kernel(x_hbm, wqkv_hbm, wo_hbm, wg_hbm, wu_hbm, wd_hbm, out_ref,
            x_v, wqkv_v, wo_v, wg_v, wu_v, wd_v,
            k_s, qt_s, vt_s, m_s, ot_s, s0, s1, w0, w1, sems):
    j = pl.program_id(0)
    s_refs = (s0, s1)
    w_refs = (w0, w1)

    def copy(src, dst, i):
        return pltpu.make_async_copy(src, dst, sems.at[i])

    x_copies = [copy(x_hbm.at[pl.ds(i * TM, TM)], x_v.at[pl.ds(i * TM, TM)], i) for i in range(NT)]
    wqkv_copy = copy(wqkv_hbm, wqkv_v, NT)
    late_copies = [copy(wo_hbm, wo_v, NT + 1), copy(wg_hbm, wg_v, NT + 2),
                   copy(wu_hbm, wu_v, NT + 3), copy(wd_hbm, wd_v, NT + 4)]

    def set_w(slot, u):
        jj = u // H
        h = u % H
        r = pl.multiple_of((h % HPG) * DH, DH)
        w_refs[slot][pl.ds(r, DH), :] = qt_s[jj, pl.ds(pl.multiple_of(h * DH, DH), DH), :]

    def clear_w(slot, u):
        r = pl.multiple_of(((u % H) % HPG) * DH, DH)
        w_refs[slot][pl.ds(r, DH), :] = jnp.zeros((DH, TQ), _bf16)

    def scores(slot, g, c):
        return jnp.dot(k_s[g, pl.ds(c * CK, CK), :], w_refs[slot][...], preferred_element_type=_f32)

    def store_scores(slot, c, s, m8):
        s_refs[slot][pl.ds(c * CK, CK), :] = s
        return jnp.maximum(m8, jnp.max(s.reshape(CK // 8, 8, TQ), axis=0))

    def pv(slot, h, c, m, l8, acc):
        s = s_refs[slot][pl.ds(c * CK, CK), :]
        p = jnp.exp2(s.reshape(CK // 8, 8, TQ) - m[None])
        l8 = l8 + jnp.sum(p, axis=0)
        vt = vt_s[h, :, pl.ds(c * CK, CK)]
        acc = acc + jnp.dot(vt, p.reshape(CK, TQ).astype(_bf16), preferred_element_type=_f32)
        return l8, acc

    def unit(u, slot, do_a, do_b):
        un = u + NS
        if do_a:
            g = (un % H) // HPG
            m8 = jnp.full((8, TQ), -jnp.inf, _f32)
        if do_b:
            h = u % H
            l8 = jnp.zeros((8, TQ), _f32)
            acc = jnp.zeros((DH, TQ), _f32)
            m = jnp.broadcast_to(m_s[slot], (8, TQ))
        hist = []
        for c in range(NC):
            if do_a:
                s = scores(slot, g, c)
            if do_b:
                mc = m
                if LAG and c >= LAG:
                    tt = hist[c - LAG]
                    mc = jnp.where(tt > jnp.inf, tt, m)
                l8, acc = pv(slot, h, c, mc, l8, acc)
                hist.append(l8)
            if do_a:
                m8 = store_scores(slot, c, s, m8)
        if do_b:
            l = jnp.sum(l8, axis=0, keepdims=True)
            ot_s[pl.ds(pl.multiple_of(h * DH, DH), DH), :] = (acc / l).astype(ot_s.dtype)
        if do_a:
            m_s[slot] = jnp.max(m8, axis=0, keepdims=True)
            clear_w(slot, un)
            set_w(slot, jnp.minimum(un + NS, NQ * H - NS + slot))

    @pl.when(j == 0)
    def _():
        x_copies[0].start()
        wqkv_copy.start()
        for w in w_refs:
            w[...] = jnp.zeros(w.shape, w.dtype)
        x_copies[0].wait()
        for cp in x_copies[1:]:
            cp.start()
        xn = _layernorm(x_v[pl.ds(0, TM), :].astype(_f32)).astype(_bf16)
        wqkv_copy.wait()
        for cp in late_copies:
            cp.start()
        for i in range(NT):
            if i + 1 < NT:
                x_copies[i + 1].wait()
                xn_next = _layernorm(x_v[pl.ds((i + 1) * TM, TM), :].astype(_f32)).astype(_bf16)
            k = jnp.dot(xn, wqkv_v[:, D:2 * D], preferred_element_type=_f32)
            for g in range(D // 128):
                k_s[g, pl.ds(i * TM, TM), :] = k[:, g * 128:(g + 1) * 128].astype(_bf16)
            qt = lax.dot_general(wqkv_v[:, 0:D], xn, (((0,), (1,)), ((), ())), preferred_element_type=_f32)
            qt_s[(i * TM) // TQ, :, pl.ds((i * TM) % TQ, TM)] = (qt * QSCALE).astype(_bf16)
            vt = lax.dot_general(wqkv_v[:, 2 * D:3 * D], xn, (((0,), (1,)), ((), ())), preferred_element_type=_f32)
            vt_s[:, :, pl.ds(i * TM, TM)] = vt.astype(_bf16).reshape(H, DH, TM)
            if i + 1 < NT:
                xn = xn_next
        for st in range(NS):
            set_w(st, st)
        for st in range(NS):
            unit(st - NS, st, True, False)

    nblk = H // NS
    last = j == NQ - 1

    def body(b, carry):
        for st in range(NS):
            unit(j * H + b * NS + st, st, True, True)
        return carry

    lax.fori_loop(0, jnp.where(last, nblk - 1, nblk), body, 0)

    @pl.when(last)
    def _():
        for st in range(NS):
            unit(NQ * H - NS + st, st, False, True)

    @pl.when(j == 0)
    def _():
        for cp in late_copies:
            cp.wait()

    attn = lax.dot_general(ot_s[...], wo_v[...], (((0,), (0,)), ((), ())), preferred_element_type=_f32)
    hres = x_v[pl.ds(pl.multiple_of(j * TQ, TQ), TQ), :].astype(_f32) + attn
    hn = _layernorm(hres).astype(_bf16)
    acc = hres
    for c in range(NF):
        g = jnp.dot(hn, wg_v[:, c * FC:(c + 1) * FC], preferred_element_type=_f32)
        u = jnp.dot(hn, wu_v[:, c * FC:(c + 1) * FC], preferred_element_type=_f32)
        a = (g * jax.nn.sigmoid(g) * u).astype(_bf16)
        acc = acc + jnp.dot(a, wd_v[c * FC:(c + 1) * FC, :], preferred_element_type=_f32)
    out_ref[...] = acc.astype(out_ref.dtype)


@jax.jit
def pallas_sequential_preLN__softmax_full_mha__swiglu_ffn__prompt_kernel(
    A_x: jax.Array,
    A_wqkv: jax.Array,
    A_wo: jax.Array,
    B_x: jax.Array,
    B_w_gate: jax.Array,
    B_w_up: jax.Array,
    B_w_down: jax.Array,
):
    del B_x
    x = A_x.reshape(S, D)
    any_spec = pl.BlockSpec(memory_space=pl.ANY)
    out = pl.pallas_call(
        _kernel,
        grid=(NQ,),
        in_specs=[any_spec] * 6,
        out_specs=pl.BlockSpec((TQ, D), lambda j: (j, 0)),
        out_shape=jax.ShapeDtypeStruct((S, D), A_x.dtype),
        scratch_shapes=[
            pltpu.VMEM((S, D), _bf16),
            pltpu.VMEM((D, 3 * D), _bf16),
            pltpu.VMEM((D, D), _bf16),
            pltpu.VMEM((D, F), _bf16),
            pltpu.VMEM((D, F), _bf16),
            pltpu.VMEM((F, D), _bf16),
            pltpu.VMEM((D // 128, S, 128), _bf16),
            pltpu.VMEM((NQ, D, TQ), _bf16),
            pltpu.VMEM((H, DH, S), _bf16),
            pltpu.VMEM((NS, 1, TQ), _f32),
            pltpu.VMEM((D, TQ), _bf16),
            pltpu.VMEM((S, TQ), _f32),
            pltpu.VMEM((S, TQ), _f32),
            pltpu.VMEM((128, TQ), _bf16),
            pltpu.VMEM((128, TQ), _bf16),
            pltpu.SemaphoreType.DMA((NT + 5,)),
        ],
        compiler_params=pltpu.CompilerParams(
            dimension_semantics=("arbitrary",),
            vmem_limit_bytes=100 * 1024 * 1024,
        ),
    )(x, A_wqkv, A_wo, B_w_gate, B_w_up, B_w_down)
    return out.reshape(A_x.shape)
```

```python
import math

import jax
import jax.numpy as jnp
from jax import lax
import jax.experimental.pallas as pl
import jax.experimental.pallas.tpu as pltpu

S, D, H, DH, F = 2048, 512, 32, 16, 1792
EPS = 1e-5

TQ = 512
NQ = S // TQ
CK = 128
NC = S // CK
NS = 4
LAG = 3
TM = 512
NT = S // TM
FC = 128
NF = F // FC
SKIPEND = 12
HEAD = 1
LNF = 0
WN = 128
B0 = 0
QSCALE = (DH ** -0.5) * math.log2(math.e)

_f32 = jnp.float32
_bf16 = jnp.bfloat16


def _layernorm(x):
    m = jnp.mean(x, axis=-1, keepdims=True)
    xc = x - m
    v = jnp.mean(xc * xc, axis=-1, keepdims=True)
    r = lax.rsqrt(v + EPS)
    if LNF:
        return x * r - m * r
    return xc * r


def _kernel(x_hbm, wqkv_hbm, wo_hbm, wg_hbm, wu_hbm, wd_hbm, out_ref,
            x_v, wq_v, wk_v, wv_v, wo_v, wg_v, wu_v, wd_v,
            k_s, qt_s, vt_s, m_s, ot_s, o_s, z_s, sems, *s_refs):
    j = pl.program_id(0)

    def copy(src, dst, i):
        return pltpu.make_async_copy(src, dst, sems.at[i])

    x_copies = [copy(x_hbm.at[pl.ds(i * TM, TM)], x_v.at[pl.ds(i * TM, TM)], i) for i in range(NT)]
    wq_copy, wk_copy, wv_copy = [copy(wqkv_hbm.at[:, pl.ds(i * D, D)], w, NT + i)
                                 for i, w in enumerate((wq_v, wk_v, wv_v))]
    late_copies = [copy(wo_hbm, wo_v, NT + 3), copy(wg_hbm, wg_v, NT + 4),
                   copy(wu_hbm, wu_v, NT + 5), copy(wd_hbm, wd_v, NT + 6)]

    def a_stage(u, slot):
        h = u & (H - 1)
        m8 = jnp.full((8, TQ), -jnp.inf, _f32)
        for c in range(NC):
            qt = qt_s[u >> 5, pl.ds(pl.multiple_of(h * DH, DH), DH), :]
            zero = jnp.zeros((DH, TQ), _bf16)
            w = jnp.concatenate([qt if i == slot else zero for i in range(NS)], axis=0)
            s = jnp.dot(k_s[h >> (NS.bit_length() - 1), pl.ds(c * CK, CK), :], w,
                        preferred_element_type=_f32)
            yield
            s_refs[slot][pl.ds(c * CK, CK), :] = s
            m8 = jnp.maximum(m8, jnp.max(s.reshape(CK // 8, 8, TQ), axis=0))
            if c == NC - 1:
                m_s[slot] = jnp.max(m8, axis=0, keepdims=True)
            yield

    def b_stage(u, slot):
        h = u & (H - 1)
        acc = z_s[...]
        m = jnp.broadcast_to(m_s[slot], (8, TQ))
        hist = [jnp.zeros((8, TQ), _f32)]
        for c in range(NC):
            s = s_refs[slot][pl.ds(c * CK, CK), :]
            mc = m
            if len(hist) > LAG:
                tt = hist[len(hist) - LAG]
                mc = jnp.where(tt < 0.0, tt, m)
            p = jnp.exp2(s.reshape(CK // 8, 8, TQ) - mc[None])
            hist.append(hist[-1] + jnp.sum(p, axis=0))
            vt = vt_s[h, :, pl.ds(c * CK, CK)]
            acc = acc + jnp.dot(vt, p.reshape(CK, TQ).astype(_bf16), preferred_element_type=_f32)
            if c == NC - 1:
                l = jnp.sum(hist[-1], axis=0, keepdims=True)
                ot_s[pl.ds(pl.multiple_of(h * DH, DH), DH), :] = (acc / l).astype(_bf16)
            yield

    @pl.when(j == 0)
    def _():
        for cp in (x_copies[0], wk_copy, x_copies[1], wq_copy, wv_copy, x_copies[2], x_copies[3], *late_copies):
            cp.start()
        z_s[...] = jnp.zeros(z_s.shape, z_s.dtype)

        def ln_tile(i):
            return _layernorm(x_v[pl.ds(i * TM, TM), :].astype(_f32)).astype(_bf16)

        def k_proj(i, xn):
            kb = jnp.dot(xn, wk_v[...], preferred_element_type=_f32).astype(_bf16)
            for g in range(H // NS):
                k_s[g, pl.ds(i * TM, TM), :] = kb[:, g * NS * DH:(g + 1) * NS * DH]

        def proj_t(w_ref, xn, nn):
            if nn:
                return jnp.dot(xn, w_ref[...], preferred_element_type=_f32).T
            return lax.dot_general(w_ref[...], xn, (((0,), (1,)), ((), ())), preferred_element_type=_f32)

        def q_proj(i, xn):
            qt = proj_t(wq_v, xn, i == 0)
            qt_s[(i * TM) // TQ, :, pl.ds((i * TM) % TQ, TM)] = (qt * QSCALE).astype(_bf16)

        def v_proj(i, xn):
            vt = proj_t(wv_v, xn, i == 0)
            vt_s[:, :, pl.ds(i * TM, TM)] = vt.astype(_bf16).reshape(H, DH, TM)

        x_copies[0].wait()
        xn0 = ln_tile(0)
        wk_copy.wait()
        k_proj(0, xn0)
        x_copies[1].wait()
        wq_copy.wait()
        xn1 = ln_tile(1)
        q_proj(0, xn0)
        k_proj(1, xn1)
        q_proj(1, xn1)
        wv_copy.wait()
        x_copies[2].wait()
        x_copies[3].wait()
        xn2 = ln_tile(2)
        v_proj(0, xn0)
        xn3 = ln_tile(3)
        v_proj(1, xn1)
        k_proj(2, xn2)
        k_proj(3, xn3)
        q_proj(2, xn2)
        v_proj(2, xn2)
        q_proj(3, xn3)
        v_proj(3, xn3)

    @pl.when((j == 0) | (j == 2) | (j == 3))
    def _():
        for st in range(NS):
            for _ in a_stage(j * H + st, st):
                pass

    def body(b, carry):
        for st in range(NS):
            u = j * H + b * NS + st
            ga, gb = a_stage(u + NS, st), b_stage(u, st)
            for _ in range(NC):
                next(ga)
                next(gb)
                next(ga)
        return carry

    nblk = H // NS
    with jax.named_scope('attnloop'):
        lax.fori_loop(0, jnp.where(j == 0, nblk, jnp.where(j == NQ, 0, nblk - 1)), body, 0)

    @pl.when(j == 0)
    def _():
        o_s[...] = ot_s[...].T
        for cp in late_copies:
            cp.wait()

    @pl.when(j >= 1)
    def _():
        def b_all():
            for st in range(NS):
                yield from b_stage(j * H + H - NS + st, st)

        gb = b_all()
        left = [NS * NC]

        def bsteps(n):
            for _ in range(min(n, left[0])):
                next(gb)
                left[0] -= 1

        nh = 2
        hr = TQ // nh
        hres = []
        for i in range(nh):
            o = o_s[i * hr:(i + 1) * hr, :]
            attn = jnp.concatenate([jnp.dot(o, wo_v[:, n * WN:(n + 1) * WN], preferred_element_type=_f32)
                                    for n in range(D // WN)], axis=1)
            r = pl.multiple_of((j - 1) * TQ + i * hr, hr)
            hres.append(x_v[pl.ds(r, hr), :].astype(_f32) + attn)
        bsteps(B0)
        hns = [_layernorm(h) for h in hres]
        hns = [h.astype(_bf16) for h in hns]
        accs = list(hres)
        nslots = 3 * NF * nh
        per = (NS * NC - B0) / (nslots - SKIPEND)
        slot = 0

        def tick():
            nonlocal slot
            slot += 1
            want = int(round(per * slot)) - int(round(per * (slot - 1)))
            bsteps(want)

        def gate(i, c):
            g = jnp.dot(hns[i], wg_v[:, c * FC:(c + 1) * FC], preferred_element_type=_f32)
            sg = g * jax.nn.sigmoid(g)
            tick()
            return sg

        def up(i, c, sg):
            u = jnp.dot(hns[i], wu_v[:, c * FC:(c + 1) * FC], preferred_element_type=_f32)
            a = (sg * u).astype(_bf16)
            tick()
            return a

        def down(i, c, a):
            accs[i] = accs[i] + jnp.dot(a, wd_v[c * FC:(c + 1) * FC, :], preferred_element_type=_f32)
            tick()

        for i in range(nh):
            for c in range(HEAD):
                down(i, c, up(i, c, gate(i, c)))
        for c in range(HEAD, NF):
            sgs = [gate(i, c) for i in range(nh)]
            acts = [up(i, c, sgs[i]) for i in range(nh)]
            for i in range(nh):
                down(i, c, acts[i])
        acc = jnp.concatenate(accs, axis=0)
        bsteps(left[0])
        o_s[...] = ot_s[...].T
        out_ref[...] = acc.astype(out_ref.dtype)


@jax.jit
def pallas_sequential_preLN__softmax_full_mha__swiglu_ffn__prompt_kernel(
    A_x: jax.Array,
    A_wqkv: jax.Array,
    A_wo: jax.Array,
    B_x: jax.Array,
    B_w_gate: jax.Array,
    B_w_up: jax.Array,
    B_w_down: jax.Array,
):
    del B_x
    x = A_x.reshape(S, D)
    any_spec = pl.BlockSpec(memory_space=pl.ANY)
    out = pl.pallas_call(
        _kernel,
        grid=(NQ + 1,),
        in_specs=[any_spec] * 6,
        out_specs=pl.BlockSpec((TQ, D), lambda j: (jnp.maximum(j - 1, 0), 0)),
        out_shape=jax.ShapeDtypeStruct((S, D), A_x.dtype),
        scratch_shapes=[
            pltpu.VMEM((S, D), _bf16),
            pltpu.VMEM((D, D), _bf16),
            pltpu.VMEM((D, D), _bf16),
            pltpu.VMEM((D, D), _bf16),
            pltpu.VMEM((D, D), _bf16),
            pltpu.VMEM((D, F), _bf16),
            pltpu.VMEM((D, F), _bf16),
            pltpu.VMEM((F, D), _bf16),
            pltpu.VMEM((H // NS, S, NS * DH), _bf16),
            pltpu.VMEM((NQ, D, TQ), _bf16),
            pltpu.VMEM((H, DH, S), _bf16),
            pltpu.VMEM((NS, 1, TQ), _f32),
            pltpu.VMEM((D, TQ), _bf16),
            pltpu.VMEM((TQ, D), _bf16),
            pltpu.VMEM((DH, TQ), _f32),
            pltpu.SemaphoreType.DMA((NT + 7,)),
        ] + [pltpu.VMEM((S, TQ), _f32)] * NS,
        compiler_params=pltpu.CompilerParams(
            dimension_semantics=("arbitrary",),
            vmem_limit_bytes=100 * 1024 * 1024,
        ),
    )(x, A_wqkv, A_wo, B_w_gate, B_w_up, B_w_down)
    return out.reshape(A_x.shape)
```

```python
import math

import jax
import jax.numpy as jnp
from jax import lax
import jax.experimental.pallas as pl
import jax.experimental.pallas.tpu as pltpu

S, D, H, DH, F = 2048, 512, 32, 16, 1792
EPS = 1e-5

TQ = 512
NQ = S // TQ
CK = 128
NC = S // CK
NS = 4
LAG = 2
FC = 128
NF = F // FC
NH = 2
HR = TQ // NH
SKIP_START = 6
SKIP_END = 12
QSCALE = (DH ** -0.5) * math.log2(math.e)

_f32 = jnp.float32
_bf16 = jnp.bfloat16


def _layernorm(x):
    m = jnp.mean(x, axis=-1, keepdims=True)
    xc = x - m
    v = jnp.mean(xc * xc, axis=-1, keepdims=True)
    return xc * lax.rsqrt(v + EPS)


def _kernel(x_hbm, wqkv_hbm, wo_hbm, wg_hbm, wu_hbm, wd_hbm, out_ref,
            x_v, wq_v, wk_v, wv_v, wo_v, wg_v, wu_v, wd_v,
            k_s, qt_s, vt_s, xn_s, m_s, ot_s, o_s, z_s, sems, *s_refs):
    j = pl.program_id(0)

    def copy(src, dst, i):
        return pltpu.make_async_copy(src, dst, sems.at[i])

    x_copies = [copy(x_hbm.at[pl.ds(i * TQ, TQ)], x_v.at[pl.ds(i * TQ, TQ)], i) for i in range(NQ)]
    wq_copy, wk_copy, wv_copy = [copy(wqkv_hbm.at[:, pl.ds(i * D, D)], w, NQ + i)
                                 for i, w in enumerate((wq_v, wk_v, wv_v))]
    late_copies = [copy(wo_hbm, wo_v, NQ + 3), copy(wg_hbm, wg_v, NQ + 4),
                   copy(wu_hbm, wu_v, NQ + 5), copy(wd_hbm, wd_v, NQ + 6)]

    def a_stage(u, slot):
        h = u & (H - 1)
        m8 = jnp.full((8, TQ), -jnp.inf, _f32)
        for c in range(NC):
            qt = qt_s[u >> 5, pl.ds(pl.multiple_of(h * DH, DH), DH), :]
            zero = jnp.zeros((DH, TQ), _bf16)
            w = jnp.concatenate([qt if i == slot else zero for i in range(NS)], axis=0)
            s = jnp.dot(k_s[h >> (NS.bit_length() - 1), pl.ds(c * CK, CK), :], w,
                        preferred_element_type=_f32)
            yield
            s_refs[slot][pl.ds(c * CK, CK), :] = s
            m8 = jnp.maximum(m8, jnp.max(s.reshape(CK // 8, 8, TQ), axis=0))
            if c == NC - 1:
                m_s[slot] = jnp.max(m8, axis=0, keepdims=True)
            yield

    def b_stage(u, slot):
        h = u & (H - 1)
        acc = z_s[...]
        m = jnp.broadcast_to(m_s[slot], (8, TQ))
        sums = [jnp.zeros((8, TQ), _f32)]
        for c in range(NC):
            s = s_refs[slot][pl.ds(c * CK, CK), :]
            mc = m
            if len(sums) > LAG:
                t = sums[len(sums) - LAG]
                mc = jnp.where(t < 0.0, t, m)
            p = jnp.exp2(s.reshape(CK // 8, 8, TQ) - mc[None])
            sums.append(sums[-1] + jnp.sum(p, axis=0))
            vt = vt_s[(c * CK) // TQ, h, :, pl.ds((c * CK) % TQ, CK)]
            acc = acc + jnp.dot(vt, p.reshape(CK, TQ).astype(_bf16), preferred_element_type=_f32)
            if c == NC - 1:
                l = jnp.sum(sums[-1], axis=0, keepdims=True)
                ot_s[pl.ds(pl.multiple_of(h * DH, DH), DH), :] = (acc / l).astype(_bf16)
            yield

    @pl.when(j == 0)
    def _():
        for cp in (x_copies[0], wk_copy, x_copies[1], wq_copy, wv_copy, x_copies[2], x_copies[3],
                   *late_copies):
            cp.start()
        z_s[...] = jnp.zeros(z_s.shape, z_s.dtype)

        def rows(i):
            return pl.ds(i * TQ if isinstance(i, int) else pl.multiple_of(i * TQ, TQ), TQ)

        def ln_tile(i):
            return _layernorm(x_v[rows(i), :].astype(_f32)).astype(_bf16)

        def k_proj(i, xn):
            kb = jnp.dot(xn, wk_v[...], preferred_element_type=_f32).astype(_bf16)
            for g in range(H // NS):
                k_s[g, rows(i), :] = kb[:, g * NS * DH:(g + 1) * NS * DH]

        def proj_t(w_ref, xn, nn):
            if nn:
                return jnp.dot(xn, w_ref[...], preferred_element_type=_f32).T
            return lax.dot_general(w_ref[...], xn, (((0,), (1,)), ((), ())),
                                   preferred_element_type=_f32)

        def q_proj(i, xn, nn=False):
            qt_s[i] = (proj_t(wq_v, xn, nn) * QSCALE).astype(_bf16)

        def v_proj(i, xn, nn=False):
            vt_s[i] = proj_t(wv_v, xn, nn).astype(_bf16).reshape(H, DH, TQ)

        x_copies[0].wait()
        xn0 = ln_tile(0)
        xn_s[0] = xn0
        wk_copy.wait()
        k_proj(0, xn0)
        x_copies[1].wait()
        wq_copy.wait()
        xn1 = ln_tile(1)
        xn_s[1] = xn1
        q_proj(0, xn0, True)
        k_proj(1, xn1)
        q_proj(1, xn1)
        wv_copy.wait()
        x_copies[2].wait()
        x_copies[3].wait()

        def qkv_body(t, carry):
            xn = ln_tile(2 + t)
            v_proj(t, xn_s[t], True)
            k_proj(2 + t, xn)
            q_proj(2 + t, xn)
            v_proj(2 + t, xn)
            return carry

        lax.fori_loop(0, 2, qkv_body, 0)

    @pl.when((j == 0) | (j == 2) | (j == 3))
    def _():
        for st in range(NS):
            for _ in a_stage(j * H + st, st):
                pass

    def body(b, carry):
        for st in range(NS):
            u = j * H + b * NS + st
            ga, gb = a_stage(u + NS, st), b_stage(u, st)
            for _ in range(NC):
                next(ga)
                next(gb)
                next(ga)
        return carry

    nblk = H // NS
    lax.fori_loop(0, jnp.where(j == 0, nblk, jnp.where(j == NQ, 0, nblk - 1)), body, 0)

    @pl.when(j == 0)
    def _():
        o_s[...] = ot_s[...].T
        for cp in late_copies:
            cp.wait()

    @pl.when(j >= 1)
    def _():
        def b_all():
            for st in range(NS):
                yield from b_stage(j * H + H - NS + st, st)

        gb = b_all()
        per = NS * NC / (3 * NF * NH - SKIP_START - SKIP_END)
        state = dict(slot=-SKIP_START, left=NS * NC)

        def b_steps(n):
            for _ in range(min(n, state["left"])):
                next(gb)
                state["left"] -= 1

        def tick():
            state["slot"] += 1
            t = state["slot"]
            if t > 0:
                b_steps(int(round(per * t)) - int(round(per * (t - 1))))

        accs = []
        for i in range(NH):
            attn = jnp.dot(o_s[i * HR:(i + 1) * HR, :], wo_v[...], preferred_element_type=_f32)
            r = pl.multiple_of((j - 1) * TQ + i * HR, HR)
            accs.append(x_v[pl.ds(r, HR), :].astype(_f32) + attn)
        hns = [_layernorm(h).astype(_bf16) for h in accs]

        def gate(i, c):
            g = jnp.dot(hns[i], wg_v[:, c * FC:(c + 1) * FC], preferred_element_type=_f32)
            sg = g * jax.nn.sigmoid(g)
            tick()
            return sg

        def up(i, c, sg):
            u = jnp.dot(hns[i], wu_v[:, c * FC:(c + 1) * FC], preferred_element_type=_f32)
            a = (sg * u).astype(_bf16)
            tick()
            return a

        def down(i, c, a):
            accs[i] = accs[i] + jnp.dot(a, wd_v[c * FC:(c + 1) * FC, :], preferred_element_type=_f32)
            tick()

        for i in range(NH):
            down(i, 0, up(i, 0, gate(i, 0)))
        for c in range(1, NF):
            sgs = [gate(i, c) for i in range(NH)]
            acts = [up(i, c, sgs[i]) for i in range(NH)]
            for i in range(NH):
                down(i, c, acts[i])
        b_steps(state["left"])
        o_s[...] = ot_s[...].T
        out_ref[...] = jnp.concatenate(accs, axis=0).astype(out_ref.dtype)


@jax.jit
def pallas_sequential_preLN__softmax_full_mha__swiglu_ffn__prompt_kernel(
    A_x: jax.Array,
    A_wqkv: jax.Array,
    A_wo: jax.Array,
    B_x: jax.Array,
    B_w_gate: jax.Array,
    B_w_up: jax.Array,
    B_w_down: jax.Array,
):
    del B_x
    x = A_x.reshape(S, D)
    any_spec = pl.BlockSpec(memory_space=pl.ANY)
    out = pl.pallas_call(
        _kernel,
        grid=(NQ + 1,),
        in_specs=[any_spec] * 6,
        out_specs=pl.BlockSpec((TQ, D), lambda j: (jnp.maximum(j - 1, 0), 0)),
        out_shape=jax.ShapeDtypeStruct((S, D), A_x.dtype),
        scratch_shapes=[
            pltpu.VMEM((S, D), _bf16),
            pltpu.VMEM((D, D), _bf16),
            pltpu.VMEM((D, D), _bf16),
            pltpu.VMEM((D, D), _bf16),
            pltpu.VMEM((D, D), _bf16),
            pltpu.VMEM((D, F), _bf16),
            pltpu.VMEM((D, F), _bf16),
            pltpu.VMEM((F, D), _bf16),
            pltpu.VMEM((H // NS, S, NS * DH), _bf16),
            pltpu.VMEM((NQ, D, TQ), _bf16),
            pltpu.VMEM((NQ, H, DH, TQ), _bf16),
            pltpu.VMEM((2, TQ, D), _bf16),
            pltpu.VMEM((NS, 1, TQ), _f32),
            pltpu.VMEM((D, TQ), _bf16),
            pltpu.VMEM((TQ, D), _bf16),
            pltpu.VMEM((DH, TQ), _f32),
            pltpu.SemaphoreType.DMA((NQ + 7,)),
        ] + [pltpu.VMEM((S, TQ), _f32)] * NS,
        compiler_params=pltpu.CompilerParams(
            dimension_semantics=("arbitrary",),
            vmem_limit_bytes=100 * 1024 * 1024,
        ),
    )(x, A_wqkv, A_wo, B_w_gate, B_w_up, B_w_down)
    return out.reshape(A_x.shape)
```
